```python
import jax
import jax.numpy as jnp

def _softmax(x, axis=-1):
    return jax.nn.softmax(x, axis=axis)

def _gelu(x):
    return jax.nn.gelu(x, approximate=True)

def _silu(x):
    return jax.nn.silu(x)

def _sigmoid(x):
    return jax.nn.sigmoid(x)

def _layernorm(x, axis=-1, eps=1e-05):
    m = jnp.mean(x, axis=axis, keepdims=True)
    v = jnp.var(x, axis=axis, keepdims=True)
    return (x - m) / jnp.sqrt(v + eps)

def _scatter_add(tgt, idx, src, axis=0):
    return tgt.at[idx].add(src)

def _segment_sum(src, seg, n):
    return jax.ops.segment_sum(src, seg, n)

class _Rng:

    def __init__(self, key):
        self._k = key

    def _next(self):
        self._k, sub = jax.random.split(self._k)
        return sub

    def normal(self, shape):
        return jax.random.normal(self._next(), shape, dtype=jnp.bfloat16)

    def randint(self, lo, hi, shape):
        return jax.random.randint(self._next(), shape, lo, hi, dtype=jnp.int32)

    def uniform(self, shape, lo=0.0, hi=1.0):
        return jax.random.uniform(self._next(), shape, jnp.bfloat16, lo, hi)

    def permutation(self, n):
        return jax.random.permutation(self._next(), n)
kernel_name = 'concat_heads__memory_aug_recurrent_mem_tr__compressed_kv_cla__prompt'

def setup_inputs():
    _rng = _Rng(jax.random.key(int.from_bytes(__import__("os").urandom(4), "little")))
    _w = lambda a: (lambda t: t.astype(jnp.bfloat16) if jnp.issubdtype(t.dtype, jnp.floating) else t)(jnp.asarray(a))

    def _A_setup():
        B, S, Dm = (1, 2048, 448)
        H, Dh = (16, 256)
        M, seg = (8, 32)
        seg = min(seg, S)
        S = S // seg * seg
        return {'x': _w((lambda *s: _rng.normal(s) * 0.05)(B, S, Dm)), 'mem0': _w((lambda *s: _rng.normal(s) * 0.05)(B, M, Dm)), 'Wq': _w((lambda *s: _rng.normal(s) * 0.05)(Dm, H, Dh) * Dm ** (-0.5)), 'Wk': _w((lambda *s: _rng.normal(s) * 0.05)(Dm, H, Dh) * Dm ** (-0.5)), 'Wv': _w((lambda *s: _rng.normal(s) * 0.05)(Dm, H, Dh) * Dm ** (-0.5)), 'Wo': _w((lambda *s: _rng.normal(s) * 0.05)(H, Dh, Dm) * (H * Dh) ** (-0.5)), 'seg_len': seg}
    _A_in = _A_setup()

    def _B_setup():
        B, H, Sq, Sk, D, M = (1, 16, 2048, 2048, 256, 448)
        Dc = 4 * D
        return {'x': _w((lambda *s: _rng.normal(s) * 0.05)(B, Sq, M)), 'c_kv': _w((lambda *s: _rng.normal(s) * 0.05)(B, Sk, Dc)), 'w_q': _w((lambda *s: _rng.normal(s) * 0.05)(M, H, D) * M ** (-0.5)), 'w_uk': _w((lambda *s: _rng.normal(s) * 0.05)(Dc, H, D) * Dc ** (-0.5)), 'w_uv': _w((lambda *s: _rng.normal(s) * 0.05)(Dc, H, D) * Dc ** (-0.5)), 'w_o': _w((lambda *s: _rng.normal(s) * 0.05)(H, D, M) * (H * D) ** (-0.5))}
    _B_in = _B_setup()
    return {'A_x': _A_in['x'], 'A_mem0': _A_in['mem0'], 'A_Wq': _A_in['Wq'], 'A_Wk': _A_in['Wk'], 'A_Wv': _A_in['Wv'], 'A_Wo': _A_in['Wo'], 'A_seg_len': _A_in['seg_len'], 'B_x': _B_in['x'], 'B_c_kv': _B_in['c_kv'], 'B_w_q': _B_in['w_q'], 'B_w_uk': _B_in['w_uk'], 'B_w_uv': _B_in['w_uv'], 'B_w_o': _B_in['w_o']}

def reference(A_x, A_mem0, A_Wq, A_Wk, A_Wv, A_Wo, A_seg_len, B_x, B_c_kv, B_w_q, B_w_uk, B_w_uv, B_w_o):

    def _A_ref(x, mem0, Wq, Wk, Wv, Wo, seg_len):
        B, S, Dm = x.shape
        H, Dh = (Wq.shape[1], Wq.shape[2])
        M = mem0.shape[1]
        scale = Dh ** (-0.5)
        n_seg = S // seg_len
        L = M + seg_len
        idx = jnp.arange(L)
        mask = (idx[:, None] < M) | (idx[:, None] >= idx[None, :])
        mem = mem0
        outs = []
        for s in range(n_seg):
            xs = x[:, s * seg_len:(s + 1) * seg_len, :].copy()
            h = jnp.concatenate([mem, xs], axis=1)
            q = jnp.einsum('btd,dhe->bhte', h, Wq)
            k = jnp.einsum('btd,dhe->bhte', h, Wk)
            v = jnp.einsum('btd,dhe->bhte', h, Wv)
            scores = jnp.einsum('bhqe,bhke->bhqk', q, k) * scale
            scores = jnp.where(mask[None, None], scores, -1000000000.0)
            p = _softmax(scores, axis=-1)
            o = jnp.einsum('bhqk,bhke->bhqe', p, v)
            o = jnp.einsum('bhte,hed->btd', o, Wo)
            mem = o[:, :M, :].copy()
            outs.append(o[:, M:, :])
        return jnp.concatenate(outs, axis=1)

    def _B_ref(x, c_kv, w_q, w_uk, w_uv, w_o):
        B, Sq, M = (x.shape[0], x.shape[1], x.shape[2])
        Sk = c_kv.shape[1]
        H, D = (w_q.shape[1], w_q.shape[2])
        q = jnp.einsum('bqm,mhd->bhqd', x, w_q)
        k = jnp.einsum('bkc,chd->bhkd', c_kv, w_uk)
        v = jnp.einsum('bkc,chd->bhkd', c_kv, w_uv)
        scores = jnp.einsum('bhqd,bhkd->bhqk', q, k) * D ** (-0.5)
        off = Sk - Sq
        qi = jnp.arange(Sq)[:, None]
        kj = jnp.arange(Sk)[None, :]
        cmask = kj <= qi + off
        scores = jnp.where(cmask[None, None], scores, -1000000000.0)
        p = _softmax(scores, axis=-1)
        ctx = jnp.einsum('bhqk,bhkd->bhqd', p, v)
        return jnp.einsum('bhqd,hdm->bqm', ctx, w_o)
    a = _A_ref(A_x, A_mem0, A_Wq, A_Wk, A_Wv, A_Wo, A_seg_len)
    b = _B_ref(B_x, B_c_kv, B_w_q, B_w_uk, B_w_uv, B_w_o)
    return jnp.concatenate([a, b], axis=-1)
```

```python
import functools
import math

import jax
import jax.numpy as jnp
import numpy as np
from jax import lax
import jax.experimental.pallas as pl
import jax.experimental.pallas.tpu as pltpu

_LOG2E = math.log2(math.e)
_NT = (((1,), (1,)), ((), ()))


def _dot(a, b):
    return jnp.dot(a, b, preferred_element_type=jnp.float32)


def _dot_nt(a, b):
    return lax.dot_general(a, b, _NT, preferred_element_type=jnp.float32)


def _head_pair(raw_ref, pair, rows, n_pairs):
    words = jnp.concatenate(
        [raw_ref[t, pl.ds(pair, rows, stride=n_pairs), :] for t in range(raw_ref.shape[0])], axis=1)
    lo = lax.bitcast_convert_type(words << 16, jnp.float32)
    hi = lax.bitcast_convert_type(words & jnp.uint32(0xFFFF0000), jnp.float32)
    return lo.astype(jnp.bfloat16), hi.astype(jnp.bfloat16)


def _kernel(xa_hbm, mem_hbm, wq_hbm, wk_hbm, wv_hbm, wo_hbm,
            xb_hbm, c_hbm, bq_hbm, buk_hbm, buv_hbm, bo_hbm,
            out_ref,
            xaT, mem0, rq, rk, rv, woT, wqkv,
            xbT, c, rbq, rbuk, rbuv, boT, acc, qs, ks, vs, xa, xb, wo, bo, sems,
            *, S, Dm, H, Dh, M, seg, Dc, BQ):
    f32, bf16 = jnp.float32, jnp.bfloat16
    HP = H // 2
    srcs = (xa_hbm, mem_hbm, wq_hbm, wk_hbm, wv_hbm, wo_hbm,
            xb_hbm, c_hbm, bq_hbm, buk_hbm, buv_hbm, bo_hbm)
    dsts = (xaT, mem0, rq, rk, rv, woT, xbT, c, rbq, rbuk, rbuv, boT)
    copies = []
    for i, (s, d) in enumerate(zip(srcs, dsts)):
        if len(d.shape) == 3:
            copies.append([pltpu.make_async_copy(s.bitcast(jnp.uint32).at[:, pl.ds(128 * t, 128)], d.at[t], sems.at[i, t])
                           for t in range(d.shape[0])])
        else:
            copies.append([pltpu.make_async_copy(s, d, sems.at[i, 0])])
    for cps in copies:
        for cp in cps:
            cp.start()

    def wait(i):
        for cp in copies[i]:
            cp.wait()

    for j, raw in enumerate((rq, rk, rv)):
        wait(2 + j)

        def relayout(i, _, raw=raw, j=j):
            lo, hi = _head_pair(raw, i, Dm, HP)
            wqkv[j * H + 2 * i] = lo
            wqkv[j * H + 2 * i + 1] = hi
            return 0

        lax.fori_loop(0, HP, relayout, 0)
    wait(0)
    xa[...] = xaT[...].T
    wait(1)
    wait(5)

    def untranspose(src, dst):
        def body(hd, _):
            dst[pl.ds(pl.multiple_of(hd * Dh, Dh), Dh), :] = src[pl.ds(pl.multiple_of(hd * Dm, Dm), Dm), :].T
            return 0
        lax.fori_loop(0, H, body, 0)

    untranspose(woT, wo)

    L = seg + 2 * M
    row = lax.broadcasted_iota(jnp.int32, (L, L), 0)
    col = lax.broadcasted_iota(jnp.int32, (L, L), 1)
    visible = (col >= seg) | (row >= seg) | (col <= row)
    fill = jnp.where(col >= seg + M, -jnp.inf, -1e9 * _LOG2E).astype(f32)
    keep = visible & (col < seg + M)
    a_scale = Dh ** -0.5 * _LOG2E

    def a_step(s, mem):
        r0 = pl.multiple_of(s * seg, seg)
        hm = jnp.concatenate([mem, jnp.zeros_like(mem)], axis=0).astype(bf16)
        h = jnp.concatenate([xa[pl.ds(r0, seg), :], hm], axis=0)
        o = jnp.zeros((L, Dm), f32)
        for hd in range(H):
            q = (_dot(h, wqkv[hd]) * a_scale).astype(bf16)
            k = _dot(h, wqkv[H + hd]).astype(bf16)
            v = _dot(h, wqkv[2 * H + hd]).astype(bf16)
            sc = jnp.where(keep, _dot_nt(q, k), fill)
            e = jnp.exp2(sc - jnp.max(sc, axis=-1, keepdims=True))
            p = e / jnp.sum(e, axis=-1, keepdims=True)
            oh = _dot(p.astype(bf16), v).astype(bf16)
            o = o + _dot(oh, wo[pl.ds(hd * Dh, Dh), :])
        out_ref[pl.ds(r0, seg), 0:Dm] = o[0:seg].astype(out_ref.dtype)
        return o[seg:seg + M].astype(bf16).astype(f32)

    with jax.named_scope('A_loop'):
        lax.fori_loop(0, S // seg, a_step, mem0[...].astype(f32))

    for i in range(6, 12):
        wait(i)
    xb[...] = xbT[...].T
    untranspose(boT, bo)
    b_scale = Dh ** -0.5 * _LOG2E
    drow = lax.broadcasted_iota(jnp.int32, (BQ, BQ), 0)
    dcol = lax.broadcasted_iota(jnp.int32, (BQ, BQ), 1)
    causal = dcol <= drow
    acc[...] = jnp.zeros_like(acc)

    def b_pair(i, _):
        wq2 = _head_pair(rbq, i, Dm, HP)
        wk2 = _head_pair(rbuk, i, Dc, HP)
        wv2 = _head_pair(rbuv, i, Dc, HP)
        for t in range(2):
            qs[...] = (_dot(xb[...], wq2[t]) * b_scale).astype(bf16)
            ks[...] = _dot(c[...], wk2[t]).astype(bf16)
            vs[...] = _dot(c[...], wv2[t]).astype(bf16)
            w_out = bo[pl.ds(pl.multiple_of((2 * i + t) * Dh, Dh), Dh), :]
            for qb in range(S // BQ):
                lo, hi = qb * BQ, (qb + 1) * BQ
                q = qs[lo:hi, :]
                sd = jnp.where(causal, _dot_nt(q, ks[lo:hi, :]), -1e9 * _LOG2E)
                m = jnp.max(sd, axis=-1, keepdims=True)
                if qb:
                    so = _dot_nt(q, ks[0:lo, :])
                    m = jnp.maximum(m, jnp.max(so, axis=-1, keepdims=True))
                ed = jnp.exp2(sd - m)
                l = jnp.sum(ed, axis=-1, keepdims=True)
                ctx = _dot(ed.astype(bf16), vs[lo:hi, :])
                if qb:
                    eo = jnp.exp2(so - m)
                    l = l + jnp.sum(eo, axis=-1, keepdims=True)
                    ctx = ctx + _dot(eo.astype(bf16), vs[0:lo, :])
                ctx = (ctx / l).astype(bf16)
                acc[lo:hi, :] += _dot(ctx, w_out)
        return 0

    with jax.named_scope('B_loop'):
        lax.fori_loop(0, HP, b_pair, 0)
    out_ref[:, Dm:2 * Dm] = acc[...].astype(out_ref.dtype)


@functools.partial(jax.jit, static_argnames=("A_seg_len",))
def pallas_concat_heads__memory_aug_recurrent_mem_tr__compressed_kv_cla__prompt_kernel(
    A_x, A_mem0, A_Wq, A_Wk, A_Wv, A_Wo, A_seg_len,
    B_x, B_c_kv, B_w_q, B_w_uk, B_w_uv, B_w_o,
):
    _, S, Dm = A_x.shape
    _, H, Dh = A_Wq.shape
    M = A_mem0.shape[1]
    Dc = B_c_kv.shape[2]
    seg = int(A_seg_len)
    bf16 = jnp.bfloat16
    BQ = 256
    args = (
        A_x.reshape(S, Dm).T, A_mem0.reshape(M, Dm),
        A_Wq.reshape(Dm * H, Dh), A_Wk.reshape(Dm * H, Dh), A_Wv.reshape(Dm * H, Dh),
        A_Wo.transpose(0, 2, 1).reshape(H * Dm, Dh),
        B_x.reshape(S, Dm).T, B_c_kv.reshape(S, Dc),
        B_w_q.reshape(Dm * H, Dh), B_w_uk.reshape(Dc * H, Dh), B_w_uv.reshape(Dc * H, Dh),
        B_w_o.transpose(0, 2, 1).reshape(H * Dm, Dh),
    )
    vm = pltpu.VMEM
    bufs = [vm((Dh // 128, a.shape[0] // 2, 128), jnp.uint32) if i in (2, 3, 4, 8, 9, 10) else vm(a.shape, bf16)
            for i, a in enumerate(args)]
    scratch = bufs[:6]
    scratch += [vm((3 * H, Dm, Dh), bf16)]
    scratch += bufs[6:]
    scratch += [vm((S, Dm), jnp.float32), vm((S, Dh), bf16), vm((S, Dh), bf16), vm((S, Dh), bf16),
                vm((S, Dm), bf16), vm((S, Dm), bf16), vm((H * Dh, Dm), bf16), vm((H * Dh, Dm), bf16),
                pltpu.SemaphoreType.DMA((12, Dh // 128))]
    out = pl.pallas_call(
        functools.partial(_kernel, S=S, Dm=Dm, H=H, Dh=Dh, M=M, seg=seg, Dc=Dc, BQ=BQ),
        out_shape=jax.ShapeDtypeStruct((S, 2 * Dm), bf16),
        in_specs=[pl.BlockSpec(memory_space=pltpu.HBM)] * 12,
        out_specs=pl.BlockSpec(memory_space=pltpu.VMEM),
        scratch_shapes=scratch,
        compiler_params=pltpu.CompilerParams(vmem_limit_bytes=120 * 1024 * 1024),
    )(*args)
    return out.reshape(1, S, 2 * Dm)
```

```python
import functools
import math

import jax
import jax.numpy as jnp
import numpy as np
from jax import lax
import jax.experimental.pallas as pl
import jax.experimental.pallas.tpu as pltpu

_LOG2E = math.log2(math.e)
_NT = (((1,), (1,)), ((), ()))


def _dot(a, b):
    return jnp.dot(a, b, preferred_element_type=jnp.float32)


def _dot_nt(a, b):
    return lax.dot_general(a, b, _NT, preferred_element_type=jnp.float32)


def _head_pair(raw_ref, pair, rows, n_pairs):
    words = jnp.concatenate(
        [raw_ref[t, pl.ds(pair, rows, stride=n_pairs), :] for t in range(raw_ref.shape[0])], axis=1)
    lo = lax.bitcast_convert_type(words << 16, jnp.float32)
    hi = lax.bitcast_convert_type(words & jnp.uint32(0xFFFF0000), jnp.float32)
    return lo.astype(jnp.bfloat16), hi.astype(jnp.bfloat16)


def _kernel(xa_hbm, mem_hbm, wq_hbm, wk_hbm, wv_hbm, wo_hbm,
            xb_hbm, c_hbm, bq_hbm, buk_hbm, buv_hbm, bo_hbm,
            out_ref,
            xaT, mem0, rq, rk, rv, woT, wqkv,
            xbT, c, rbq, rbuk, rbuv, boT, acc, qs, ks, vs, xa, xb, wo, bo, sems,
            *, S, Dm, H, Dh, M, seg, Dc, BQ):
    f32, bf16 = jnp.float32, jnp.bfloat16
    HP = H // 2
    srcs = (xa_hbm, mem_hbm, wq_hbm, wk_hbm, wv_hbm, wo_hbm,
            xb_hbm, c_hbm, bq_hbm, buk_hbm, buv_hbm, bo_hbm)
    dsts = (xaT, mem0, rq, rk, rv, woT, xbT, c, rbq, rbuk, rbuv, boT)
    copies = []
    for i, (s, d) in enumerate(zip(srcs, dsts)):
        if len(d.shape) == 3:
            copies.append([pltpu.make_async_copy(s.bitcast(jnp.uint32).at[:, pl.ds(128 * t, 128)], d.at[t], sems.at[i, t])
                           for t in range(d.shape[0])])
        else:
            copies.append([pltpu.make_async_copy(s, d, sems.at[i, 0])])
    for cps in copies:
        for cp in cps:
            cp.start()

    def wait(i):
        for cp in copies[i]:
            cp.wait()

    for j, raw in enumerate((rq, rk, rv)):
        wait(2 + j)

        def relayout(i, _, raw=raw, j=j):
            lo, hi = _head_pair(raw, i, Dm, HP)
            wqkv[j * H + 2 * i] = lo
            wqkv[j * H + 2 * i + 1] = hi
            return 0

        lax.fori_loop(0, HP, relayout, 0)
    wait(0)
    xa[...] = xaT[...].T
    wait(1)
    wait(5)

    def untranspose(src, dst):
        def body(hd, _):
            dst[pl.ds(pl.multiple_of(hd * Dh, Dh), Dh), :] = src[pl.ds(pl.multiple_of(hd * Dm, Dm), Dm), :].T
            return 0
        lax.fori_loop(0, H, body, 0)

    untranspose(woT, wo)

    L = seg + 2 * M
    row = lax.broadcasted_iota(jnp.int32, (L, L), 0)
    col = lax.broadcasted_iota(jnp.int32, (L, L), 1)
    visible = (col >= seg) | (row >= seg) | (col <= row)
    fill = jnp.where(col >= seg + M, -jnp.inf, -1e9 * _LOG2E).astype(f32)
    keep = visible & (col < seg + M)
    a_scale = Dh ** -0.5 * _LOG2E

    def a_step(s, mem):
        r0 = pl.multiple_of(s * seg, seg)
        hm = jnp.concatenate([mem, jnp.zeros_like(mem)], axis=0).astype(bf16)
        h = jnp.concatenate([xa[pl.ds(r0, seg), :], hm], axis=0)
        qkv, ps, ohs = {}, {}, {}

        def proj(hd):
            q = (_dot(h, wqkv[hd]) * a_scale).astype(bf16)
            k = _dot(h, wqkv[H + hd]).astype(bf16)
            v = _dot(h, wqkv[2 * H + hd]).astype(bf16)
            qkv[hd] = (q, k, v)

        def scores(hd):
            q, k, _ = qkv[hd]
            sc = jnp.where(keep, _dot_nt(q, k), fill)
            e = jnp.exp2(sc - jnp.max(sc, axis=-1, keepdims=True))
            ps[hd] = (e / jnp.sum(e, axis=-1, keepdims=True)).astype(bf16)

        def context(hd):
            ohs[hd] = _dot(ps[hd], qkv[hd][2]).astype(bf16)

        for t in range(H):
            proj(t)
            if t >= 1:
                scores(t - 1)
            if t >= 2:
                context(t - 2)
        o = None
        for t in range(H):
            part = _dot(ohs[t], wo[pl.ds(t * Dh, Dh), :])
            o = part if o is None else o + part
            if t == 1:
                scores(H - 1)
            if t == 3:
                context(H - 2)
            if t == 6:
                context(H - 1)
        out_ref[pl.ds(r0, seg), 0:Dm] = o[0:seg].astype(out_ref.dtype)
        return o[seg:seg + M].astype(bf16).astype(f32)

    with jax.named_scope('A_loop'):
        lax.fori_loop(0, S // seg, a_step, mem0[...].astype(f32))

    for i in range(6, 12):
        wait(i)
    xb[...] = xbT[...].T
    untranspose(boT, bo)
    b_scale = Dh ** -0.5 * _LOG2E
    drow = lax.broadcasted_iota(jnp.int32, (BQ, BQ), 0)
    dcol = lax.broadcasted_iota(jnp.int32, (BQ, BQ), 1)
    causal = dcol <= drow
    acc[...] = jnp.zeros_like(acc)

    def b_pair(i, _):
        wq2 = _head_pair(rbq, i, Dm, HP)
        wk2 = _head_pair(rbuk, i, Dc, HP)
        wv2 = _head_pair(rbuv, i, Dc, HP)
        for t in range(2):
            qs[...] = (_dot(xb[...], wq2[t]) * b_scale).astype(bf16)
            ks[...] = _dot(c[...], wk2[t]).astype(bf16)
            vs[...] = _dot(c[...], wv2[t]).astype(bf16)
            w_out = bo[pl.ds(pl.multiple_of((2 * i + t) * Dh, Dh), Dh), :]
            for qb in range(S // BQ):
                lo, hi = qb * BQ, (qb + 1) * BQ
                q = qs[lo:hi, :]
                sd = jnp.where(causal, _dot_nt(q, ks[lo:hi, :]), -1e9 * _LOG2E)
                m = jnp.max(sd, axis=-1, keepdims=True)
                if qb:
                    so = _dot_nt(q, ks[0:lo, :])
                    m = jnp.maximum(m, jnp.max(so, axis=-1, keepdims=True))
                ed = jnp.exp2(sd - m)
                l = jnp.sum(ed, axis=-1, keepdims=True)
                ctx = _dot(ed.astype(bf16), vs[lo:hi, :])
                if qb:
                    eo = jnp.exp2(so - m)
                    l = l + jnp.sum(eo, axis=-1, keepdims=True)
                    ctx = ctx + _dot(eo.astype(bf16), vs[0:lo, :])
                ctx = (ctx / l).astype(bf16)
                acc[lo:hi, :] += _dot(ctx, w_out)
        return 0

    with jax.named_scope('B_loop'):
        lax.fori_loop(0, HP, b_pair, 0)
    out_ref[:, Dm:2 * Dm] = acc[...].astype(out_ref.dtype)


@functools.partial(jax.jit, static_argnames=("A_seg_len",))
def pallas_concat_heads__memory_aug_recurrent_mem_tr__compressed_kv_cla__prompt_kernel(
    A_x, A_mem0, A_Wq, A_Wk, A_Wv, A_Wo, A_seg_len,
    B_x, B_c_kv, B_w_q, B_w_uk, B_w_uv, B_w_o,
):
    _, S, Dm = A_x.shape
    _, H, Dh = A_Wq.shape
    M = A_mem0.shape[1]
    Dc = B_c_kv.shape[2]
    seg = int(A_seg_len)
    bf16 = jnp.bfloat16
    BQ = 256
    args = (
        A_x.reshape(S, Dm).T, A_mem0.reshape(M, Dm),
        A_Wq.reshape(Dm * H, Dh), A_Wk.reshape(Dm * H, Dh), A_Wv.reshape(Dm * H, Dh),
        A_Wo.transpose(0, 2, 1).reshape(H * Dm, Dh),
        B_x.reshape(S, Dm).T, B_c_kv.reshape(S, Dc),
        B_w_q.reshape(Dm * H, Dh), B_w_uk.reshape(Dc * H, Dh), B_w_uv.reshape(Dc * H, Dh),
        B_w_o.transpose(0, 2, 1).reshape(H * Dm, Dh),
    )
    vm = pltpu.VMEM
    bufs = [vm((Dh // 128, a.shape[0] // 2, 128), jnp.uint32) if i in (2, 3, 4, 8, 9, 10) else vm(a.shape, bf16)
            for i, a in enumerate(args)]
    scratch = bufs[:6]
    scratch += [vm((3 * H, Dm, Dh), bf16)]
    scratch += bufs[6:]
    scratch += [vm((S, Dm), jnp.float32), vm((S, Dh), bf16), vm((S, Dh), bf16), vm((S, Dh), bf16),
                vm((S, Dm), bf16), vm((S, Dm), bf16), vm((H * Dh, Dm), bf16), vm((H * Dh, Dm), bf16),
                pltpu.SemaphoreType.DMA((12, Dh // 128))]
    out = pl.pallas_call(
        functools.partial(_kernel, S=S, Dm=Dm, H=H, Dh=Dh, M=M, seg=seg, Dc=Dc, BQ=BQ),
        out_shape=jax.ShapeDtypeStruct((S, 2 * Dm), bf16),
        in_specs=[pl.BlockSpec(memory_space=pltpu.HBM)] * 12,
        out_specs=pl.BlockSpec(memory_space=pltpu.VMEM),
        scratch_shapes=scratch,
        compiler_params=pltpu.CompilerParams(vmem_limit_bytes=120 * 1024 * 1024),
    )(*args)
    return out.reshape(1, S, 2 * Dm)
```

```python
import functools
import math

import jax
import jax.numpy as jnp
import numpy as np
from jax import lax
import jax.experimental.pallas as pl
import jax.experimental.pallas.tpu as pltpu

_LOG2E = math.log2(math.e)
_NT = (((1,), (1,)), ((), ()))


def _dot(a, b):
    return jnp.dot(a, b, preferred_element_type=jnp.float32)


def _dot_nt(a, b):
    return lax.dot_general(a, b, _NT, preferred_element_type=jnp.float32)


def _head_pair(raw_ref, pair, rows, n_pairs):
    words = jnp.concatenate(
        [raw_ref[t, pl.ds(pair, rows, stride=n_pairs), :] for t in range(raw_ref.shape[0])], axis=1)
    lo = lax.bitcast_convert_type(words << 16, jnp.float32)
    hi = lax.bitcast_convert_type(words & jnp.uint32(0xFFFF0000), jnp.float32)
    return lo.astype(jnp.bfloat16), hi.astype(jnp.bfloat16)


def _kernel(xa_hbm, mem_hbm, wq_hbm, wk_hbm, wv_hbm, wo_hbm,
            xb_hbm, c_hbm, bq_hbm, buk_hbm, buv_hbm, bo_hbm,
            out_ref,
            xaT, mem0, rq, rk, rv, woT, wqkv,
            xbT, c, rbq, rbuk, rbuv, boT, accT, qall, ks, vs, xa, xb, wo, sems,
            *, S, Dm, H, Dh, M, seg, Dc, BQ):
    f32, bf16 = jnp.float32, jnp.bfloat16
    HP = H // 2
    srcs = (xa_hbm, mem_hbm, wq_hbm, wk_hbm, wv_hbm, wo_hbm,
            xb_hbm, c_hbm, bq_hbm, buk_hbm, buv_hbm, bo_hbm)
    dsts = (xaT, mem0, rq, rk, rv, woT, xbT, c, rbq, rbuk, rbuv, boT)
    copies = []
    for i, (s, d) in enumerate(zip(srcs, dsts)):
        if len(d.shape) == 3:
            copies.append([pltpu.make_async_copy(s.bitcast(jnp.uint32).at[:, pl.ds(128 * t, 128)],
                                                 d.at[t], sems.at[i, t])
                           for t in range(d.shape[0])])
        else:
            copies.append([pltpu.make_async_copy(s, d, sems.at[i, 0])])

    def start(*ids):
        for i in ids:
            for cp in copies[i]:
                cp.start()

    def wait(*ids):
        for i in ids:
            for cp in copies[i]:
                cp.wait()

    b_scale = Dh ** -0.5 * _LOG2E
    start(6, 8)
    wait(6)
    start(0, 1, 2, 3, 4, 5)
    xb[...] = xbT[...].T
    wait(8)

    def q_pair(i):
        for t, w in enumerate(_head_pair(rbq, i, Dm, HP)):
            qall[2 * i + t] = (_dot(xb[...], w) * b_scale).astype(bf16)

    def q_first(i, _):
        q_pair(i)
        return 0

    def q_second(i, _):
        q_pair(HP // 2 + i)
        for pair in (2 * i, 2 * i + 1):
            for j, raw in enumerate((rq, rk, rv)):
                lo, hi = _head_pair(raw, pair, Dm, HP)
                wqkv[j * H + 2 * pair] = lo
                wqkv[j * H + 2 * pair + 1] = hi
            for hd in (2 * pair, 2 * pair + 1):
                wo[pl.ds(pl.multiple_of(hd * Dh, Dh), Dh), :] = (
                    woT[pl.ds(pl.multiple_of(hd * Dm, Dm), Dm), :].T)
        return 0

    with jax.named_scope("Q_proj"):
        lax.fori_loop(0, HP // 2, q_first, 0)
        wait(0, 1, 2, 3, 4, 5)
        start(7, 9, 10, 11)
        lax.fori_loop(0, HP // 2, q_second, 0)
        xa[...] = xaT[...].T

    L = seg + M
    row = lax.broadcasted_iota(jnp.int32, (2 * L, 2 * L), 0)
    col = lax.broadcasted_iota(jnp.int32, (2 * L, 2 * L), 1)
    same_head = (row >= L) == (col >= L)
    r = jnp.where(row >= L, row - L, row)
    cc = jnp.where(col >= L, col - L, col)
    keep = same_head & ((cc >= seg) | (r >= seg) | (cc <= r))
    fill = jnp.where(same_head, -1e9 * _LOG2E, -jnp.inf).astype(f32)
    a_scale = Dh ** -0.5 * _LOG2E

    def a_step(s, mem):
        r0 = pl.multiple_of(s * seg, seg)
        pad = jnp.zeros((M, Dh), f32)
        hm = jnp.concatenate([mem, jnp.zeros_like(mem)], axis=0).astype(bf16)
        h = jnp.concatenate([xa[pl.ds(r0, seg), :], hm], axis=0)
        qkv, ps, ohs = {}, {}, {}

        def proj(g):
            def both(j):
                return jnp.concatenate(
                    [_dot(h, wqkv[j * H + 2 * g + t])[0:L] for t in range(2)], axis=0)
            qkv[g] = ((both(0) * a_scale).astype(bf16), both(1).astype(bf16), both(2).astype(bf16))

        def scores(g):
            q, k, _ = qkv[g]
            sc = jnp.where(keep, _dot_nt(q, k), fill)
            e = jnp.exp2(sc - jnp.max(sc, axis=-1, keepdims=True))
            ps[g] = (e / jnp.sum(e, axis=-1, keepdims=True)).astype(bf16)

        def context(g):
            o2 = _dot(ps[g], qkv[g][2])
            for t in range(2):
                ohs[2 * g + t] = jnp.concatenate([o2[t * L:(t + 1) * L], pad], axis=0).astype(bf16)

        for g in range(HP):
            proj(g)
            if g >= 1:
                scores(g - 1)
            if g >= 2:
                context(g - 2)
        o = None
        for t in range(H):
            part = _dot(ohs[t], wo[pl.ds(t * Dh, Dh), :])
            o = part if o is None else o + part
            if t == 1:
                scores(HP - 1)
            if t == 3:
                context(HP - 2)
            if t == 6:
                context(HP - 1)
        out_ref[pl.ds(r0, seg), 0:Dm] = o[0:seg].astype(out_ref.dtype)
        return o[seg:seg + M].astype(bf16).astype(f32)

    with jax.named_scope("A_loop"):
        lax.fori_loop(0, S // seg, a_step, mem0[...].astype(f32))

    wait(7, 9, 10, 11)
    HB = BQ // 2
    masked = -1e9 * _LOG2E
    vis_a = (lax.broadcasted_iota(jnp.int32, (BQ, HB), 1)
             <= lax.broadcasted_iota(jnp.int32, (BQ, HB), 0))
    vis_b = vis_a[0:HB]
    accT[...] = jnp.zeros_like(accT)

    def b_pair(i, _):
        wk2 = _head_pair(rbuk, i, Dc, HP)
        wv2 = _head_pair(rbuv, i, Dc, HP)
        for t in range(2):
            hd = 2 * i + t
            ks[...] = _dot(c[...], wk2[t]).astype(bf16)
            vs[...] = _dot(c[...], wv2[t]).astype(bf16)
            w_out = boT[pl.ds(pl.multiple_of(hd * Dm, Dm), Dm), :]
            sc, ctxs = {}, {}

            def scores(qb):
                lo, mid, hi = qb * BQ, qb * BQ + HB, (qb + 1) * BQ
                q = qall[hd, lo:hi, :]
                sa = jnp.where(vis_a, _dot_nt(q, ks[lo:mid, :]), masked)
                sb = jnp.where(vis_b, _dot_nt(q[HB:], ks[mid:hi, :]), masked)
                so = _dot_nt(q, ks[0:lo, :]) if qb else None
                sc[qb] = (sa, sb, so)

            def context(qb):
                lo, mid, hi = qb * BQ, qb * BQ + HB, (qb + 1) * BQ
                sa, sb, so = sc[qb]
                top = jnp.concatenate([sa[0:HB], jnp.maximum(sa[HB:], sb)], axis=0)
                m = jnp.max(top, axis=-1, keepdims=True)
                if qb:
                    m = jnp.maximum(m, jnp.max(so, axis=-1, keepdims=True))
                ea = jnp.exp2(sa - m)
                eb = jnp.exp2(sb - m[HB:])
                l = jnp.sum(jnp.concatenate([ea[0:HB], ea[HB:] + eb], axis=0), axis=-1, keepdims=True)
                ctx = _dot(ea.astype(bf16), vs[lo:mid, :])
                cb = _dot(eb.astype(bf16), vs[mid:hi, :])
                ctx = jnp.concatenate([ctx[0:HB], ctx[HB:] + cb], axis=0)
                if qb:
                    eo = jnp.exp2(so - m)
                    l = l + jnp.sum(eo, axis=-1, keepdims=True)
                    ctx = ctx + _dot(eo.astype(bf16), vs[0:lo, :])
                ctxs[qb] = (ctx / l).astype(bf16)

            def project(qb):
                accT[:, qb * BQ:(qb + 1) * BQ] += _dot_nt(w_out, ctxs[qb])

            NQ = S // BQ
            scores(0)
            for qb in range(NQ):
                if qb + 1 < NQ:
                    scores(qb + 1)
                context(qb)
                if qb >= 1:
                    project(qb - 1)
            project(NQ - 1)
        return 0

    with jax.named_scope("B_loop"):
        lax.fori_loop(0, HP, b_pair, 0)
    out_ref[:, Dm:2 * Dm] = accT[...].T.astype(out_ref.dtype)


@functools.partial(jax.jit, static_argnames=("A_seg_len",))
def pallas_concat_heads__memory_aug_recurrent_mem_tr__compressed_kv_cla__prompt_kernel(
    A_x, A_mem0, A_Wq, A_Wk, A_Wv, A_Wo, A_seg_len,
    B_x, B_c_kv, B_w_q, B_w_uk, B_w_uv, B_w_o,
):
    _, S, Dm = A_x.shape
    _, H, Dh = A_Wq.shape
    M = A_mem0.shape[1]
    Dc = B_c_kv.shape[2]
    seg = int(A_seg_len)
    bf16 = jnp.bfloat16
    BQ = 256
    args = (
        A_x.reshape(S, Dm).T, A_mem0.reshape(M, Dm),
        A_Wq.reshape(Dm * H, Dh), A_Wk.reshape(Dm * H, Dh), A_Wv.reshape(Dm * H, Dh),
        A_Wo.transpose(0, 2, 1).reshape(H * Dm, Dh),
        B_x.reshape(S, Dm).T, B_c_kv.reshape(S, Dc),
        B_w_q.reshape(Dm * H, Dh), B_w_uk.reshape(Dc * H, Dh), B_w_uv.reshape(Dc * H, Dh),
        B_w_o.transpose(0, 2, 1).reshape(H * Dm, Dh),
    )
    vm = pltpu.VMEM
    bufs = [vm((Dh // 128, a.shape[0] // 2, 128), jnp.uint32) if i in (2, 3, 4, 8, 9, 10) else vm(a.shape, bf16)
            for i, a in enumerate(args)]
    scratch = bufs[:6]
    scratch += [vm((3 * H, Dm, Dh), bf16)]
    scratch += bufs[6:]
    scratch += [vm((Dm, S), jnp.float32), vm((H, S, Dh), bf16), vm((S, Dh), bf16), vm((S, Dh), bf16),
                vm((S, Dm), bf16), vm((S, Dm), bf16), vm((H * Dh, Dm), bf16),
                pltpu.SemaphoreType.DMA((12, Dh // 128))]
    out = pl.pallas_call(
        functools.partial(_kernel, S=S, Dm=Dm, H=H, Dh=Dh, M=M, seg=seg, Dc=Dc, BQ=BQ),
        out_shape=jax.ShapeDtypeStruct((S, 2 * Dm), bf16),
        in_specs=[pl.BlockSpec(memory_space=pltpu.HBM)] * 12,
        out_specs=pl.BlockSpec(memory_space=pltpu.VMEM),
        scratch_shapes=scratch,
        compiler_params=pltpu.CompilerParams(vmem_limit_bytes=120 * 1024 * 1024),
    )(*args)
    return out.reshape(1, S, 2 * Dm)
```

```python
import functools
import math

import jax
import jax.numpy as jnp
import numpy as np
from jax import lax
import jax.experimental.pallas as pl
import jax.experimental.pallas.tpu as pltpu

_LOG2E = math.log2(math.e)
_NT = (((1,), (1,)), ((), ()))


def _dot(a, b):
    return jnp.dot(a, b, preferred_element_type=jnp.float32)


def _dot_nt(a, b):
    return lax.dot_general(a, b, _NT, preferred_element_type=jnp.float32)


def _head_pair(raw_ref, pair, rows, n_pairs):
    words = jnp.concatenate(
        [raw_ref[t, pl.ds(pair, rows, stride=n_pairs), :] for t in range(raw_ref.shape[0])], axis=1)
    lo = lax.bitcast_convert_type(words << 16, jnp.float32)
    hi = lax.bitcast_convert_type(words & jnp.uint32(0xFFFF0000), jnp.float32)
    return lo.astype(jnp.bfloat16), hi.astype(jnp.bfloat16)


def _kernel(xa_hbm, mem_hbm, wq_hbm, wk_hbm, wv_hbm, wo_hbm,
            xb_hbm, c_hbm, bq_hbm, buk_hbm, buv_hbm, bo_hbm,
            out_hbm,
            xaT, mem0, rq, rk, rv, woT, wqkv,
            xbT, c, rbq, rbuk, rbuv, boT, accT, qall, ks, vs, xa, xb, wo, out_ref, sems, osems,
            *, S, Dm, H, Dh, M, seg, Dc, BQ):
    f32, bf16 = jnp.float32, jnp.bfloat16
    HP = H // 2
    srcs = (xa_hbm, mem_hbm, wq_hbm, wk_hbm, wv_hbm, wo_hbm,
            xb_hbm, c_hbm, bq_hbm, buk_hbm, buv_hbm, bo_hbm)
    dsts = (xaT, mem0, rq, rk, rv, woT, xbT, c, rbq, rbuk, rbuv, boT)
    copies = []
    for i, (s, d) in enumerate(zip(srcs, dsts)):
        if len(d.shape) == 3:
            copies.append([pltpu.make_async_copy(s.bitcast(jnp.uint32).at[:, pl.ds(128 * t, 128)],
                                                 d.at[t], sems.at[i, t])
                           for t in range(d.shape[0])])
        else:
            copies.append([pltpu.make_async_copy(s, d, sems.at[i, 0])])

    def start(*ids):
        for i in ids:
            for cp in copies[i]:
                cp.start()

    def wait(*ids):
        for i in ids:
            for cp in copies[i]:
                cp.wait()

    b_scale = Dh ** -0.5 * _LOG2E
    start(6, 8)
    wait(6)
    xb[...] = xbT[...].T
    wait(8)
    start(2, 3, 4, 5, 0, 1)

    def q_pair(i):
        for t, w in enumerate(_head_pair(rbq, i, Dm, HP)):
            qall[2 * i + t] = (_dot(xb[...], w) * b_scale).astype(bf16)

    def q_first(i, _):
        q_pair(i)
        return 0

    def q_second(i, _):
        q_pair(HP - 2 + i)
        for pair in [i * (HP // 2) + u for u in range(HP // 2)]:
            for j, raw in enumerate((rq, rk, rv)):
                lo, hi = _head_pair(raw, pair, Dm, HP)
                wqkv[j * H + 2 * pair] = lo
                wqkv[j * H + 2 * pair + 1] = hi
            for hd in (2 * pair, 2 * pair + 1):
                wo[pl.ds(pl.multiple_of(hd * Dh, Dh), Dh), :] = (
                    woT[pl.ds(pl.multiple_of(hd * Dm, Dm), Dm), :].T)
        return 0

    with jax.named_scope("Q_proj"):
        lax.fori_loop(0, HP - 2, q_first, 0)
        wait(0, 1, 2, 3, 4, 5)
        start(7, 9, 10, 11)
        lax.fori_loop(0, 2, q_second, 0)
        xa[...] = xaT[...].T

    L = seg + M
    row = lax.broadcasted_iota(jnp.int32, (2 * L, 2 * L), 0)
    col = lax.broadcasted_iota(jnp.int32, (2 * L, 2 * L), 1)
    same_head = (row >= L) == (col >= L)
    r = jnp.where(row >= L, row - L, row)
    cc = jnp.where(col >= L, col - L, col)
    keep = same_head & ((cc >= seg) | (r >= seg) | (cc <= r))
    fill = jnp.where(same_head, -1e9 * _LOG2E, -jnp.inf).astype(f32)
    a_scale = Dh ** -0.5 * _LOG2E

    def a_step(s, mem):
        r0 = pl.multiple_of(s * seg, seg)
        pad = jnp.zeros((M, Dh), f32)
        hm = jnp.concatenate([mem, jnp.zeros_like(mem)], axis=0).astype(bf16)
        h = jnp.concatenate([xa[pl.ds(r0, seg), :], hm], axis=0)
        qkv, ps, ohs = {}, {}, {}

        def proj(g):
            def both(j):
                return jnp.concatenate(
                    [_dot(h, wqkv[j * H + 2 * g + t])[0:L] for t in range(2)], axis=0)
            qkv[g] = ((both(0) * a_scale).astype(bf16), both(1).astype(bf16), both(2).astype(bf16))

        def scores(g):
            q, k, _ = qkv[g]
            sc = jnp.where(keep, _dot_nt(q, k), fill)
            e = jnp.exp2(sc - jnp.max(sc, axis=-1, keepdims=True))
            ps[g] = (e / jnp.sum(e, axis=-1, keepdims=True)).astype(bf16)

        def context(g):
            o2 = _dot(ps[g], qkv[g][2])
            for t in range(2):
                ohs[2 * g + t] = jnp.concatenate([o2[t * L:(t + 1) * L], pad], axis=0).astype(bf16)

        for g in range(HP):
            proj(g)
            if g >= 1:
                scores(g - 1)
            if g >= 2:
                context(g - 2)
        o = None
        for t in range(H):
            part = _dot(ohs[t], wo[pl.ds(t * Dh, Dh), :])
            o = part if o is None else o + part
            if t == 1:
                scores(HP - 1)
            if t == 3:
                context(HP - 2)
            if t == 6:
                context(HP - 1)
        out_ref[pl.ds(r0, seg), 0:Dm] = o[0:seg].astype(out_ref.dtype)
        return o[seg:seg + M].astype(bf16).astype(f32)

    with jax.named_scope("A_loop"):
        lax.fori_loop(0, S // seg, a_step, mem0[...].astype(f32))

    split = Dm // 128 * 128
    outs = [pltpu.make_async_copy(out_ref.at[:, pl.ds(0, split)], out_hbm.at[:, pl.ds(0, split)], osems.at[4])]
    outs[0].start()
    wait(7, 9, 10, 11)
    HB = BQ // 2
    masked = -1e9 * _LOG2E
    vis_a = (lax.broadcasted_iota(jnp.int32, (BQ, HB), 1)
             <= lax.broadcasted_iota(jnp.int32, (BQ, HB), 0))
    vis_b = vis_a[0:HB]
    accT[...] = jnp.zeros_like(accT)

    def b_pair(i, _):
        wk2 = _head_pair(rbuk, i, Dc, HP)
        wv2 = _head_pair(rbuv, i, Dc, HP)
        for t in range(2):
            hd = 2 * i + t
            ks[...] = _dot(c[...], wk2[t]).astype(bf16)
            vs[...] = _dot(c[...], wv2[t]).astype(bf16)
            w_out = boT[pl.ds(pl.multiple_of(hd * Dm, Dm), Dm), :]
            sc, ctxs, mx = {}, {}, {}
            NQ = S // BQ
            CK = 256

            def chunks(qb):
                return [(j * CK, min((j + 1) * CK, qb * BQ)) for j in range(-(-qb * BQ // CK))]

            def fold(x, op):
                r = x[:, 0:128]
                for j in range(1, x.shape[1] // 128):
                    r = op(r, x[:, j * 128:(j + 1) * 128])
                return r

            def scores(qb):
                lo, mid, hi = qb * BQ, qb * BQ + HB, (qb + 1) * BQ
                q = qall[hd, lo:hi, :]
                sa = jnp.where(vis_a, _dot_nt(q, ks[lo:mid, :]), masked)
                sb = jnp.where(vis_b, _dot_nt(q[HB:], ks[mid:hi, :]), masked)
                top = jnp.concatenate([sa[0:HB], jnp.maximum(sa[HB:], sb)], axis=0)
                so = []
                yield
                for u, w in chunks(qb):
                    x = _dot_nt(q, ks[u:w, :])
                    top = jnp.maximum(top, fold(x, jnp.maximum))
                    so.append(x)
                    yield
                sc[qb] = (sa, sb, so, jnp.max(top, axis=-1, keepdims=True))

            def context(qb):
                lo, mid, hi = qb * BQ, qb * BQ + HB, (qb + 1) * BQ
                sa, sb, so, m = sc[qb]
                ea = jnp.exp2(sa - m)
                eb = jnp.exp2(sb - m[HB:])
                l = jnp.concatenate([ea[0:HB], ea[HB:] + eb], axis=0)
                ctx = _dot(ea.astype(bf16), vs[lo:mid, :])
                cb = _dot(eb.astype(bf16), vs[mid:hi, :])
                ctx = jnp.concatenate([ctx[0:HB], ctx[HB:] + cb], axis=0)
                yield
                for (u, w), x in zip(chunks(qb), so):
                    e = jnp.exp2(x - m)
                    l = l + fold(e, jnp.add)
                    ctx = ctx + _dot(e.astype(bf16), vs[u:w, :])
                    yield
                ctxs[qb] = (ctx / jnp.sum(l, axis=-1, keepdims=True)).astype(bf16)

            def project(qb):
                accT[:, qb * BQ:(qb + 1) * BQ] += _dot_nt(w_out, ctxs[qb])
                yield

            def weave(*gens):
                gens = list(gens)
                while gens:
                    for g in list(gens):
                        if next(g, "end") == "end":
                            gens.remove(g)

            order = list(range(NQ))[::-1]
            for step in range(NQ + 2):
                weave(*[fn(order[step - d]) for fn, d in ((scores,0),(context,1),(project,2)) if 0 <= step - d < NQ])
        return 0

    with jax.named_scope("B_loop"):
        lax.fori_loop(0, HP, b_pair, 0)
    for j in range(4):
        rows = pl.ds(j * (S // 4), S // 4)
        out_ref[rows, Dm:2 * Dm] = accT[:, rows].T.astype(out_ref.dtype)
        cols = pl.ds(split, 2 * Dm - split)
        outs.append(pltpu.make_async_copy(out_ref.at[rows, cols], out_hbm.at[rows, cols], osems.at[j]))
        outs[-1].start()
    for cp in outs:
        cp.wait()


@functools.partial(jax.jit, static_argnames=("A_seg_len",))
def pallas_concat_heads__memory_aug_recurrent_mem_tr__compressed_kv_cla__prompt_kernel(
    A_x, A_mem0, A_Wq, A_Wk, A_Wv, A_Wo, A_seg_len,
    B_x, B_c_kv, B_w_q, B_w_uk, B_w_uv, B_w_o,
):
    _, S, Dm = A_x.shape
    _, H, Dh = A_Wq.shape
    M = A_mem0.shape[1]
    Dc = B_c_kv.shape[2]
    seg = int(A_seg_len)
    bf16 = jnp.bfloat16
    BQ = 256
    args = (
        A_x.reshape(S, Dm).T, A_mem0.reshape(M, Dm),
        A_Wq.reshape(Dm * H, Dh), A_Wk.reshape(Dm * H, Dh), A_Wv.reshape(Dm * H, Dh),
        A_Wo.transpose(0, 2, 1).reshape(H * Dm, Dh),
        B_x.reshape(S, Dm).T, B_c_kv.reshape(S, Dc),
        B_w_q.reshape(Dm * H, Dh), B_w_uk.reshape(Dc * H, Dh), B_w_uv.reshape(Dc * H, Dh),
        B_w_o.transpose(0, 2, 1).reshape(H * Dm, Dh),
    )
    vm = pltpu.VMEM
    bufs = [vm((Dh // 128, a.shape[0] // 2, 128), jnp.uint32) if i in (2, 3, 4, 8, 9, 10) else vm(a.shape, bf16)
            for i, a in enumerate(args)]
    scratch = bufs[:6]
    scratch += [vm((3 * H, Dm, Dh), bf16)]
    scratch += bufs[6:]
    scratch += [vm((Dm, S), jnp.float32), vm((H, S, Dh), bf16), vm((S, Dh), bf16), vm((S, Dh), bf16),
                vm((S, Dm), bf16), vm((S, Dm), bf16), vm((H * Dh, Dm), bf16),
                vm((S, 2 * Dm), bf16),
                pltpu.SemaphoreType.DMA((12, Dh // 128)), pltpu.SemaphoreType.DMA((5,))]
    out = pl.pallas_call(
        functools.partial(_kernel, S=S, Dm=Dm, H=H, Dh=Dh, M=M, seg=seg, Dc=Dc, BQ=BQ),
        out_shape=jax.ShapeDtypeStruct((S, 2 * Dm), bf16),
        in_specs=[pl.BlockSpec(memory_space=pltpu.HBM)] * 12,
        out_specs=pl.BlockSpec(memory_space=pltpu.HBM),
        scratch_shapes=scratch,
        compiler_params=pltpu.CompilerParams(vmem_limit_bytes=120 * 1024 * 1024),
    )(*args)
    return out.reshape(1, S, 2 * Dm)
```

```python
import functools
import math

import jax
import jax.numpy as jnp
import numpy as np
from jax import lax
import jax.experimental.pallas as pl
import jax.experimental.pallas.tpu as pltpu

_LOG2E = math.log2(math.e)
_NT = (((1,), (1,)), ((), ()))


def _dot(a, b):
    return jnp.dot(a, b, preferred_element_type=jnp.float32)


def _dot_nt(a, b):
    return lax.dot_general(a, b, _NT, preferred_element_type=jnp.float32)


def _head_pair(raw_ref, pair, rows, n_pairs):
    words = jnp.concatenate(
        [raw_ref[t, pl.ds(pair, rows, stride=n_pairs), :] for t in range(raw_ref.shape[0])], axis=1)
    lo = lax.bitcast_convert_type(words << 16, jnp.float32)
    hi = lax.bitcast_convert_type(words & jnp.uint32(0xFFFF0000), jnp.float32)
    return lo.astype(jnp.bfloat16), hi.astype(jnp.bfloat16)


def _kernel(xa_hbm, mem_hbm, wq_hbm, wk_hbm, wv_hbm, wo_hbm,
            xb_hbm, c_hbm, bq_hbm, buk_hbm, buv_hbm, bo_hbm,
            out_hbm,
            xaT, mem0, rq, rk, rv, woT, wqkv,
            xbT, c, rbq, rbuk, rbuv, boT, accT, qall, ks, vs, xa, xb, wo, w4, wo4, wql, out_ref, sems, osems,
            *, S, Dm, H, Dh, M, seg, Dc, BQ):
    f32, bf16 = jnp.float32, jnp.bfloat16
    HP = H // 2
    DK = Dm // 128 * 128
    srcs = (xa_hbm, mem_hbm, wq_hbm, wk_hbm, wv_hbm, wo_hbm,
            xb_hbm, c_hbm, bq_hbm, buk_hbm, buv_hbm, bo_hbm)
    dsts = (xaT, mem0, rq, rk, rv, woT, xbT, c, rbq, rbuk, rbuv, boT)
    copies = []
    for i, (s, d) in enumerate(zip(srcs, dsts)):
        if len(d.shape) == 3:
            copies.append([pltpu.make_async_copy(s.bitcast(jnp.uint32).at[:, pl.ds(128 * t, 128)],
                                                 d.at[t], sems.at[i, t])
                           for t in range(d.shape[0])])
        else:
            copies.append([pltpu.make_async_copy(s, d, sems.at[i, 0])])

    def start(*ids):
        for i in ids:
            for cp in copies[i]:
                cp.start()

    def wait(*ids):
        for i in ids:
            for cp in copies[i]:
                cp.wait()

    b_scale = Dh ** -0.5 * _LOG2E
    start(6, 8)
    wait(6)
    xb[...] = xbT[...].T
    wait(8)
    start(2, 3, 4, 5, 0, 1)

    def q_pair(i):
        for t, w in enumerate(_head_pair(rbq, i, Dm, HP)):
            qall[2 * i + t] = (_dot(xb[...], w) * b_scale).astype(bf16)

    def q_first(i, _):
        q_pair(i)
        return 0

    def q_second(i, _):
        q_pair(HP - 4 + i)
        wql[2 * i], wql[2 * i + 1] = _head_pair(rbq, HP - 2 + i, Dm, HP)
        for pair in [i * (HP // 2) + u for u in range(HP // 2)]:
            for j, raw in enumerate((rq, rk, rv)):
                for t, w in enumerate(_head_pair(raw, pair, Dm, HP)):
                    wqkv[j * H + 2 * pair + t] = w[0:DK]
                    w4[j * H + 2 * pair + t] = jnp.concatenate([w[DK:, 0:128], w[DK:, 128:]], axis=0)
            tails = []
            for hd in (2 * pair, 2 * pair + 1):
                wo[pl.ds(pl.multiple_of(hd * Dh, Dh), Dh), :] = (
                    woT[pl.ds(pl.multiple_of(hd * Dm, Dm), DK), :].T)
                tails.append(woT[pl.ds(pl.multiple_of(hd * Dm + DK, Dm - DK), Dm - DK), :])
            wo4[pair] = jnp.concatenate(tails, axis=0).T
        return 0

    with jax.named_scope("Q_proj"):
        lax.fori_loop(0, HP - 4, q_first, 0)
        wait(0, 1, 2, 3, 4, 5)
        start(7, 9, 10, 11)
        lax.fori_loop(0, 2, q_second, 0)
        xa[...] = xaT[...].T

    L = seg + M
    row = lax.broadcasted_iota(jnp.int32, (2 * L, 2 * L), 0)
    col = lax.broadcasted_iota(jnp.int32, (2 * L, 2 * L), 1)
    same_head = (row >= L) == (col >= L)
    r = jnp.where(row >= L, row - L, row)
    cc = jnp.where(col >= L, col - L, col)
    keep = same_head & ((cc >= seg) | (r >= seg) | (cc <= r))
    fill = jnp.where(same_head, -1e9 * _LOG2E, -jnp.inf).astype(f32)
    a_scale = Dh ** -0.5 * _LOG2E

    def a_step(s, mem):
        r0 = pl.multiple_of(s * seg, seg)
        pad = jnp.zeros((M, Dh), f32)
        hm = jnp.concatenate([mem, jnp.zeros_like(mem)], axis=0).astype(bf16)
        h = jnp.concatenate([xa[pl.ds(r0, seg), 0:DK], hm[:, 0:DK]], axis=0)
        h4 = jnp.concatenate([xa[pl.ds(r0, seg), DK:Dm].astype(f32), mem[:, DK:Dm]], axis=0)
        z4 = jnp.zeros_like(h4)
        h4 = jnp.concatenate([jnp.concatenate([h4, z4], axis=1),
                              jnp.concatenate([z4, h4], axis=1)], axis=0).astype(bf16)
        qkv, ps, ohs = {}, {}, {}

        def proj(g):
            def one(n):
                tail = _dot(h4, w4[n])
                return _dot(h, wqkv[n])[0:L] + jnp.concatenate([tail[0:L], tail[L:]], axis=1)

            def both(j):
                return jnp.concatenate([one(j * H + 2 * g + t) for t in range(2)], axis=0)
            qkv[g] = ((both(0) * a_scale).astype(bf16), both(1).astype(bf16), both(2).astype(bf16))

        def scores(g):
            q, k, _ = qkv[g]
            sc = jnp.where(keep, _dot_nt(q, k), fill)
            e = jnp.exp2(sc - jnp.max(sc, axis=-1, keepdims=True))
            ps[g] = (e / jnp.sum(e, axis=-1, keepdims=True)).astype(bf16)

        def context(g):
            o2 = _dot(ps[g], qkv[g][2])
            ohs["pair", g] = o2.astype(bf16)
            for t in range(2):
                ohs[2 * g + t] = jnp.concatenate([o2[t * L:(t + 1) * L], pad], axis=0).astype(bf16)

        for g in range(HP):
            proj(g)
            if g >= 1:
                scores(g - 1)
            if g >= 2:
                context(g - 2)
        o = o4 = None
        for t in range(H):
            part = _dot(ohs[t], wo[pl.ds(t * Dh, Dh), :])
            o = part if o is None else o + part
            if t % 2:
                part = _dot(ohs["pair", t // 2], wo4[t // 2])
                o4 = part if o4 is None else o4 + part
            if t == 1:
                scores(HP - 1)
            if t == 3:
                context(HP - 2)
            if t == 6:
                context(HP - 1)
        nrow = 4 * S // (S // seg)
        late = s // (S // nrow)
        rows = pl.ds(pl.multiple_of(s % (S // nrow) * nrow, nrow), nrow)
        qall[H - 4 + late, rows, :] = (_dot(xb[rows, :], wql[late]) * b_scale).astype(bf16)
        o = jnp.concatenate([o[0:L], o4[0:L, 0:Dm - DK] + o4[L:, Dm - DK:]], axis=1)
        out_ref[pl.ds(r0, seg), 0:Dm] = o[0:seg].astype(out_ref.dtype)
        return o[seg:seg + M].astype(bf16).astype(f32)

    with jax.named_scope("A_loop"):
        lax.fori_loop(0, S // seg, a_step, mem0[...].astype(f32))

    split = Dm // 128 * 128
    outs = [pltpu.make_async_copy(out_ref.at[:, pl.ds(0, split)], out_hbm.at[:, pl.ds(0, split)], osems.at[4])]
    outs[0].start()
    wait(7, 9, 10, 11)
    HB = BQ // 2
    masked = -1e9 * _LOG2E
    vis_a = (lax.broadcasted_iota(jnp.int32, (BQ, HB), 1)
             <= lax.broadcasted_iota(jnp.int32, (BQ, HB), 0))
    vis_b = vis_a[0:HB]
    accT[...] = jnp.zeros_like(accT)

    def b_pair(i, _):
        wk2 = _head_pair(rbuk, i, Dc, HP)
        wv2 = _head_pair(rbuv, i, Dc, HP)
        for t in range(2):
            hd = 2 * i + t
            ks[...] = _dot(c[...], wk2[t]).astype(bf16)
            vs[...] = _dot(c[...], wv2[t]).astype(bf16)
            w_out = boT[pl.ds(pl.multiple_of(hd * Dm, Dm), Dm), :]
            sc, ctxs, mx = {}, {}, {}
            NQ = S // BQ
            CK = 256

            def chunks(qb):
                return [(j * CK, min((j + 1) * CK, qb * BQ)) for j in range(-(-qb * BQ // CK))]

            def fold(x, op):
                r = x[:, 0:128]
                for j in range(1, x.shape[1] // 128):
                    r = op(r, x[:, j * 128:(j + 1) * 128])
                return r

            def scores(qb):
                lo, mid, hi = qb * BQ, qb * BQ + HB, (qb + 1) * BQ
                q = qall[hd, lo:hi, :]
                sa = jnp.where(vis_a, _dot_nt(q, ks[lo:mid, :]), masked)
                sb = jnp.where(vis_b, _dot_nt(q[HB:], ks[mid:hi, :]), masked)
                top = jnp.concatenate([sa[0:HB], jnp.maximum(sa[HB:], sb)], axis=0)
                so = []
                yield
                for u, w in chunks(qb):
                    x = _dot_nt(q, ks[u:w, :])
                    top = jnp.maximum(top, fold(x, jnp.maximum))
                    so.append(x)
                    yield
                sc[qb] = (sa, sb, so, jnp.max(top, axis=-1, keepdims=True))

            def context(qb):
                lo, mid, hi = qb * BQ, qb * BQ + HB, (qb + 1) * BQ
                sa, sb, so, m = sc[qb]
                ea = jnp.exp2(sa - m)
                eb = jnp.exp2(sb - m[HB:])
                l = jnp.concatenate([ea[0:HB], ea[HB:] + eb], axis=0)
                ctx = _dot(ea.astype(bf16), vs[lo:mid, :])
                cb = _dot(eb.astype(bf16), vs[mid:hi, :])
                ctx = jnp.concatenate([ctx[0:HB], ctx[HB:] + cb], axis=0)
                yield
                for (u, w), x in zip(chunks(qb), so):
                    e = jnp.exp2(x - m)
                    l = l + fold(e, jnp.add)
                    ctx = ctx + _dot(e.astype(bf16), vs[u:w, :])
                    yield
                ctxs[qb] = (ctx / jnp.sum(l, axis=-1, keepdims=True)).astype(bf16)

            def project(qb):
                accT[:, qb * BQ:(qb + 1) * BQ] += _dot_nt(w_out, ctxs[qb])
                yield

            def weave(*gens):
                gens = list(gens)
                while gens:
                    for g in list(gens):
                        if next(g, "end") == "end":
                            gens.remove(g)

            order = list(range(NQ))[::-1]
            for step in range(NQ + 2):
                weave(*[fn(order[step - d]) for fn, d in ((scores,0),(context,1),(project,2)) if 0 <= step - d < NQ])
        return 0

    with jax.named_scope("B_loop"):
        lax.fori_loop(0, HP, b_pair, 0)
    for j in range(4):
        rows = pl.ds(j * (S // 4), S // 4)
        out_ref[rows, Dm:2 * Dm] = accT[:, rows].T.astype(out_ref.dtype)
        cols = pl.ds(split, 2 * Dm - split)
        outs.append(pltpu.make_async_copy(out_ref.at[rows, cols], out_hbm.at[rows, cols], osems.at[j]))
        outs[-1].start()
    for cp in outs:
        cp.wait()


@functools.partial(jax.jit, static_argnames=("A_seg_len",))
def pallas_concat_heads__memory_aug_recurrent_mem_tr__compressed_kv_cla__prompt_kernel(
    A_x, A_mem0, A_Wq, A_Wk, A_Wv, A_Wo, A_seg_len,
    B_x, B_c_kv, B_w_q, B_w_uk, B_w_uv, B_w_o,
):
    _, S, Dm = A_x.shape
    _, H, Dh = A_Wq.shape
    M = A_mem0.shape[1]
    Dc = B_c_kv.shape[2]
    seg = int(A_seg_len)
    bf16 = jnp.bfloat16
    BQ = 256
    DK = Dm // 128 * 128
    args = (
        A_x.reshape(S, Dm).T, A_mem0.reshape(M, Dm),
        A_Wq.reshape(Dm * H, Dh), A_Wk.reshape(Dm * H, Dh), A_Wv.reshape(Dm * H, Dh),
        A_Wo.transpose(0, 2, 1).reshape(H * Dm, Dh),
        B_x.reshape(S, Dm).T, B_c_kv.reshape(S, Dc),
        B_w_q.reshape(Dm * H, Dh), B_w_uk.reshape(Dc * H, Dh), B_w_uv.reshape(Dc * H, Dh),
        B_w_o.transpose(0, 2, 1).reshape(H * Dm, Dh),
    )
    vm = pltpu.VMEM
    bufs = [vm((Dh // 128, a.shape[0] // 2, 128), jnp.uint32) if i in (2, 3, 4, 8, 9, 10) else vm(a.shape, bf16)
            for i, a in enumerate(args)]
    scratch = bufs[:6]
    scratch += [vm((3 * H, DK, Dh), bf16)]
    scratch += bufs[6:]
    scratch += [vm((Dm, S), jnp.float32), vm((H, S, Dh), bf16), vm((S, Dh), bf16), vm((S, Dh), bf16),
                vm((S, Dm), bf16), vm((S, Dm), bf16), vm((H * Dh, DK), bf16),
                vm((3 * H, 128, 128), bf16), vm((H // 2, Dh, 128), bf16), vm((4, Dm, Dh), bf16),
                vm((S, 2 * Dm), bf16),
                pltpu.SemaphoreType.DMA((12, Dh // 128)), pltpu.SemaphoreType.DMA((5,))]
    out = pl.pallas_call(
        functools.partial(_kernel, S=S, Dm=Dm, H=H, Dh=Dh, M=M, seg=seg, Dc=Dc, BQ=BQ),
        out_shape=jax.ShapeDtypeStruct((S, 2 * Dm), bf16),
        in_specs=[pl.BlockSpec(memory_space=pltpu.HBM)] * 12,
        out_specs=pl.BlockSpec(memory_space=pltpu.HBM),
        scratch_shapes=scratch,
        compiler_params=pltpu.CompilerParams(vmem_limit_bytes=120 * 1024 * 1024),
    )(*args)
    return out.reshape(1, S, 2 * Dm)
```

```python
import functools
import math

import jax
import jax.numpy as jnp
import numpy as np
from jax import lax
import jax.experimental.pallas as pl
import jax.experimental.pallas.tpu as pltpu

_LOG2E = math.log2(math.e)
_NT = (((1,), (1,)), ((), ()))


def _dot(a, b):
    return jnp.dot(a, b, preferred_element_type=jnp.float32)


def _dot_nt(a, b):
    return lax.dot_general(a, b, _NT, preferred_element_type=jnp.float32)


def _head_pair(raw_ref, pair, rows, n_pairs):
    words = jnp.concatenate(
        [raw_ref[t, pl.ds(pair, rows, stride=n_pairs), :] for t in range(raw_ref.shape[0])], axis=1)
    lo = lax.bitcast_convert_type(words << 16, jnp.float32)
    hi = lax.bitcast_convert_type(words & jnp.uint32(0xFFFF0000), jnp.float32)
    return lo.astype(jnp.bfloat16), hi.astype(jnp.bfloat16)


def _kernel(xa_hbm, mem_hbm, wq_hbm, wk_hbm, wv_hbm, wo_hbm,
            xb_hbm, c_hbm, bq_hbm, buk_hbm, buv_hbm, bo_hbm,
            out_hbm,
            xaT, mem0, rq, rk, rv, woT, wqkv,
            xbT, c, rbq, rbuk, rbuv, boT, accT, qall, ks, vs, xa, xb, wo, w4, wo4, wql, out_ref, sems, osems,
            *, S, Dm, H, Dh, M, seg, Dc, BQ):
    f32, bf16 = jnp.float32, jnp.bfloat16
    HP = H // 2
    DK = Dm // 128 * 128
    srcs = (xa_hbm, mem_hbm, wq_hbm, wk_hbm, wv_hbm, wo_hbm,
            xb_hbm, c_hbm, bq_hbm, buk_hbm, buv_hbm, bo_hbm)
    dsts = (xaT, mem0, rq, rk, rv, woT, xbT, c, rbq, rbuk, rbuv, boT)
    copies = []
    for i, (s, d) in enumerate(zip(srcs, dsts)):
        if len(d.shape) == 3:
            copies.append([pltpu.make_async_copy(s.bitcast(jnp.uint32).at[:, pl.ds(128 * t, 128)],
                                                 d.at[t], sems.at[i, t])
                           for t in range(d.shape[0])])
        else:
            copies.append([pltpu.make_async_copy(s, d, sems.at[i, 0])])

    def start(*ids):
        for i in ids:
            for cp in copies[i]:
                cp.start()

    def wait(*ids):
        for i in ids:
            for cp in copies[i]:
                cp.wait()

    b_scale = Dh ** -0.5 * _LOG2E
    start(6, 8)
    wait(6)
    xb[...] = xbT[...].T
    wait(8)
    start(2, 3, 4, 5, 0, 1)

    def q_pair(i):
        for t, w in enumerate(_head_pair(rbq, i, Dm, HP)):
            qall[2 * i + t] = (_dot(xb[...], w) * b_scale).astype(bf16)

    def q_first(i, _):
        q_pair(i)
        return 0

    def q_second(i, _):
        q_pair(HP - 4 + i)
        wql[2 * i], wql[2 * i + 1] = _head_pair(rbq, HP - 2 + i, Dm, HP)
        for pair in [i * (HP // 2) + u for u in range(HP // 2)]:
            for j, raw in enumerate((rq, rk, rv)):
                for t, w in enumerate(_head_pair(raw, pair, Dm, HP)):
                    wqkv[j * H + 2 * pair + t] = w[0:DK]
                    w4[j * H + 2 * pair + t] = jnp.concatenate([w[DK:, 0:128], w[DK:, 128:]], axis=0)
            tails = []
            for hd in (2 * pair, 2 * pair + 1):
                wo[pl.ds(pl.multiple_of(hd * Dh, Dh), Dh), :] = (
                    woT[pl.ds(pl.multiple_of(hd * Dm, Dm), DK), :].T)
                tails.append(woT[pl.ds(pl.multiple_of(hd * Dm + DK, Dm - DK), Dm - DK), :])
            wo4[pair] = jnp.concatenate(tails, axis=0).T
        return 0

    lax.fori_loop(0, HP - 4, q_first, 0)
    wait(0, 1, 2, 3, 4, 5)
    start(7, 9, 10, 11)
    lax.fori_loop(0, 2, q_second, 0)
    xa[...] = xaT[...].T

    L = seg + M
    row = lax.broadcasted_iota(jnp.int32, (2 * L, 2 * L), 0)
    col = lax.broadcasted_iota(jnp.int32, (2 * L, 2 * L), 1)
    same_head = (row >= L) == (col >= L)
    r = jnp.where(row >= L, row - L, row)
    cc = jnp.where(col >= L, col - L, col)
    keep = same_head & ((cc >= seg) | (r >= seg) | (cc <= r))
    fill = jnp.where(same_head, -1e9 * _LOG2E, -jnp.inf).astype(f32)
    a_scale = Dh ** -0.5 * _LOG2E

    def a_step(s, mem):
        r0 = pl.multiple_of(s * seg, seg)
        pad = jnp.zeros((M, Dh), f32)
        hm = jnp.concatenate([mem, jnp.zeros_like(mem)], axis=0).astype(bf16)
        h = jnp.concatenate([xa[pl.ds(r0, seg), 0:DK], hm[:, 0:DK]], axis=0)
        h4 = jnp.concatenate([xa[pl.ds(r0, seg), DK:Dm].astype(f32), mem[:, DK:Dm]], axis=0)
        z4 = jnp.zeros_like(h4)
        h4 = jnp.concatenate([jnp.concatenate([h4, z4], axis=1),
                              jnp.concatenate([z4, h4], axis=1)], axis=0).astype(bf16)
        qkv, ps, ohs = {}, {}, {}

        def proj(g):
            def one(n):
                tail = _dot(h4, w4[n])
                return _dot(h, wqkv[n])[0:L] + jnp.concatenate([tail[0:L], tail[L:]], axis=1)

            def both(j):
                return jnp.concatenate([one(j * H + 2 * g + t) for t in range(2)], axis=0)
            qkv[g] = ((both(0) * a_scale).astype(bf16), both(1).astype(bf16), both(2).astype(bf16))

        def scores(g):
            q, k, _ = qkv[g]
            sc = jnp.where(keep, _dot_nt(q, k), fill)
            e = jnp.exp2(sc - jnp.max(sc, axis=-1, keepdims=True))
            ps[g] = (e / jnp.sum(e, axis=-1, keepdims=True)).astype(bf16)

        def context(g):
            o2 = _dot(ps[g], qkv[g][2])
            ohs["pair", g] = o2.astype(bf16)
            for t in range(2):
                ohs[2 * g + t] = jnp.concatenate([o2[t * L:(t + 1) * L], pad], axis=0).astype(bf16)

        for g in range(HP):
            proj(g)
            if g >= 1:
                scores(g - 1)
            if g >= 2:
                context(g - 2)
        o = o4 = None
        for t in range(H):
            part = _dot(ohs[t], wo[pl.ds(t * Dh, Dh), :])
            o = part if o is None else o + part
            if t % 2:
                part = _dot(ohs["pair", t // 2], wo4[t // 2])
                o4 = part if o4 is None else o4 + part
            if t == 1:
                scores(HP - 1)
            if t == 3:
                context(HP - 2)
            if t == 6:
                context(HP - 1)
        nrow = 4 * S // (S // seg)
        late = s // (S // nrow)
        rows = pl.ds(pl.multiple_of(s % (S // nrow) * nrow, nrow), nrow)
        qall[H - 4 + late, rows, :] = (_dot(xb[rows, :], wql[late]) * b_scale).astype(bf16)
        o = jnp.concatenate([o[0:L], o4[0:L, 0:Dm - DK] + o4[L:, Dm - DK:]], axis=1)
        out_ref[pl.ds(r0, seg), 0:Dm] = o[0:seg].astype(out_ref.dtype)
        return o[seg:seg + M].astype(bf16).astype(f32)

    lax.fori_loop(0, S // seg, a_step, mem0[...].astype(f32))

    split = Dm // 128 * 128
    outs = [pltpu.make_async_copy(out_ref.at[:, pl.ds(0, split)], out_hbm.at[:, pl.ds(0, split)], osems.at[4])]
    outs[0].start()
    wait(7, 9, 10, 11)
    HB = BQ // 2
    masked = -1e9 * _LOG2E
    vis_a = (lax.broadcasted_iota(jnp.int32, (BQ, HB), 1)
             <= lax.broadcasted_iota(jnp.int32, (BQ, HB), 0))
    vis_b = vis_a[0:HB]
    accT[...] = jnp.zeros_like(accT)

    def b_pair(i, _):
        wk2 = _head_pair(rbuk, i, Dc, HP)
        wv2 = _head_pair(rbuv, i, Dc, HP)
        for t in range(2):
            hd = 2 * i + t
            ks[...] = _dot(c[...], wk2[t]).astype(bf16)
            vs[...] = _dot(c[...], wv2[t]).astype(bf16)
            w_out = boT[pl.ds(pl.multiple_of(hd * Dm, Dm), Dm), :]
            sc, ctxs, mx = {}, {}, {}
            NQ = S // BQ
            CK = BQ

            def chunks(qb):
                return [(j * CK, min((j + 1) * CK, qb * BQ)) for j in range(-(-qb * BQ // CK))]

            def fold(x, op):
                r = x[:, 0:128]
                for j in range(1, x.shape[1] // 128):
                    r = op(r, x[:, j * 128:(j + 1) * 128])
                return r

            def scores(qb):
                lo, mid, hi = qb * BQ, qb * BQ + HB, (qb + 1) * BQ
                q = qall[hd, lo:hi, :]
                sa = jnp.where(vis_a, _dot_nt(q, ks[lo:mid, :]), masked)
                sb = jnp.where(vis_b, _dot_nt(q[HB:], ks[mid:hi, :]), masked)
                top = jnp.concatenate([sa[0:HB], jnp.maximum(sa[HB:], sb)], axis=0)
                so = []
                yield
                for u, w in chunks(qb):
                    x = _dot_nt(q, ks[u:w, :])
                    top = jnp.maximum(top, fold(x, jnp.maximum))
                    so.append(x)
                    yield
                sc[qb] = (sa, sb, so, jnp.max(top, axis=-1, keepdims=True))

            def context(qb):
                lo, mid, hi = qb * BQ, qb * BQ + HB, (qb + 1) * BQ
                sa, sb, so, m = sc[qb]
                ea = jnp.exp2(sa - m)
                eb = jnp.exp2(sb - m[HB:])
                l = jnp.concatenate([ea[0:HB], ea[HB:] + eb], axis=0)
                ctx = _dot(ea.astype(bf16), vs[lo:mid, :])
                cb = _dot(eb.astype(bf16), vs[mid:hi, :])
                ctx = jnp.concatenate([ctx[0:HB], ctx[HB:] + cb], axis=0)
                yield
                for (u, w), x in zip(chunks(qb), so):
                    e = jnp.exp2(x - m)
                    l = l + fold(e, jnp.add)
                    ctx = ctx + _dot(e.astype(bf16), vs[u:w, :])
                    yield
                ctxs[qb] = (ctx / jnp.sum(l, axis=-1, keepdims=True)).astype(bf16)

            def project(qb):
                for _ in range(max(qb - 1, 0) // 2):
                    yield
                accT[:, qb * BQ:(qb + 1) * BQ] += _dot_nt(w_out, ctxs[qb])
                yield

            def weave(*gens):
                gens = list(gens)
                while gens:
                    for g in list(gens):
                        if next(g, "end") == "end":
                            gens.remove(g)

            order = list(range(NQ))[::-1]
            for step in range(NQ + 2):
                weave(*[fn(order[step - d]) for fn, d in ((scores, 0), (context, 1), (project, 2)) if 0 <= step - d < NQ])
        return 0

    lax.fori_loop(0, HP, b_pair, 0)
    for j in range(4):
        rows = pl.ds(j * (S // 4), S // 4)
        out_ref[rows, Dm:2 * Dm] = accT[:, rows].T.astype(out_ref.dtype)
        cols = pl.ds(split, 2 * Dm - split)
        outs.append(pltpu.make_async_copy(out_ref.at[rows, cols], out_hbm.at[rows, cols], osems.at[j]))
        outs[-1].start()
    for cp in outs:
        cp.wait()


@functools.partial(jax.jit, static_argnames=("A_seg_len",))
def pallas_concat_heads__memory_aug_recurrent_mem_tr__compressed_kv_cla__prompt_kernel(
    A_x, A_mem0, A_Wq, A_Wk, A_Wv, A_Wo, A_seg_len,
    B_x, B_c_kv, B_w_q, B_w_uk, B_w_uv, B_w_o,
):
    _, S, Dm = A_x.shape
    _, H, Dh = A_Wq.shape
    M = A_mem0.shape[1]
    Dc = B_c_kv.shape[2]
    seg = int(A_seg_len)
    bf16 = jnp.bfloat16
    BQ = 256
    DK = Dm // 128 * 128
    args = (
        A_x.reshape(S, Dm).T, A_mem0.reshape(M, Dm),
        A_Wq.reshape(Dm * H, Dh), A_Wk.reshape(Dm * H, Dh), A_Wv.reshape(Dm * H, Dh),
        A_Wo.transpose(0, 2, 1).reshape(H * Dm, Dh),
        B_x.reshape(S, Dm).T, B_c_kv.reshape(S, Dc),
        B_w_q.reshape(Dm * H, Dh), B_w_uk.reshape(Dc * H, Dh), B_w_uv.reshape(Dc * H, Dh),
        B_w_o.transpose(0, 2, 1).reshape(H * Dm, Dh),
    )
    vm = pltpu.VMEM
    bufs = [vm((Dh // 128, a.shape[0] // 2, 128), jnp.uint32) if i in (2, 3, 4, 8, 9, 10) else vm(a.shape, bf16)
            for i, a in enumerate(args)]
    scratch = bufs[:6]
    scratch += [vm((3 * H, DK, Dh), bf16)]
    scratch += bufs[6:]
    scratch += [vm((Dm, S), jnp.float32), vm((H, S, Dh), bf16), vm((S, Dh), bf16), vm((S, Dh), bf16),
                vm((S, Dm), bf16), vm((S, Dm), bf16), vm((H * Dh, DK), bf16),
                vm((3 * H, 128, 128), bf16), vm((H // 2, Dh, 128), bf16), vm((4, Dm, Dh), bf16),
                vm((S, 2 * Dm), bf16),
                pltpu.SemaphoreType.DMA((12, Dh // 128)), pltpu.SemaphoreType.DMA((5,))]
    out = pl.pallas_call(
        functools.partial(_kernel, S=S, Dm=Dm, H=H, Dh=Dh, M=M, seg=seg, Dc=Dc, BQ=BQ),
        out_shape=jax.ShapeDtypeStruct((S, 2 * Dm), bf16),
        in_specs=[pl.BlockSpec(memory_space=pltpu.HBM)] * 12,
        out_specs=pl.BlockSpec(memory_space=pltpu.HBM),
        scratch_shapes=scratch,
        compiler_params=pltpu.CompilerParams(vmem_limit_bytes=120 * 1024 * 1024),
    )(*args)
    return out.reshape(1, S, 2 * Dm)
```

```python
import functools
import math

import jax
import jax.numpy as jnp
import numpy as np
from jax import lax
import jax.experimental.pallas as pl
import jax.experimental.pallas.tpu as pltpu

_LOG2E = math.log2(math.e)
_NT = (((1,), (1,)), ((), ()))


def _dot(a, b):
    return jnp.dot(a, b, preferred_element_type=jnp.float32)


def _dot_nt(a, b):
    return lax.dot_general(a, b, _NT, preferred_element_type=jnp.float32)


def _head_pair(raw_ref, pair, rows, n_pairs):
    words = jnp.concatenate(
        [raw_ref[t, pl.ds(pair, rows, stride=n_pairs), :] for t in range(raw_ref.shape[0])], axis=1)
    lo = lax.bitcast_convert_type(words << 16, jnp.float32)
    hi = lax.bitcast_convert_type(words & jnp.uint32(0xFFFF0000), jnp.float32)
    return lo.astype(jnp.bfloat16), hi.astype(jnp.bfloat16)


def _kernel(xa_hbm, mem_hbm, wq_hbm, wk_hbm, wv_hbm, wo_hbm,
            xb_hbm, c_hbm, bq_hbm, buk_hbm, buv_hbm, bo_hbm,
            out_hbm,
            xaT, mem0, rq, rk, rv, woT, wqkv,
            xbT, c, rbq, rbuk, rbuv, boT, accT, qall, ks, vs, xa, xb, wo, w4, wo4, wql, out_ref, sems, osems,
            *, S, Dm, H, Dh, M, seg, Dc, BQ):
    f32, bf16 = jnp.float32, jnp.bfloat16
    HP = H // 2
    DK = Dm // 128 * 128
    srcs = (xa_hbm, mem_hbm, wq_hbm, wk_hbm, wv_hbm, wo_hbm,
            xb_hbm, c_hbm, bq_hbm, buk_hbm, buv_hbm, bo_hbm)
    dsts = (xaT, mem0, rq, rk, rv, woT, xbT, c, rbq, rbuk, rbuv, boT)
    copies = []
    for i, (s, d) in enumerate(zip(srcs, dsts)):
        if len(d.shape) == 3:
            copies.append([pltpu.make_async_copy(s.bitcast(jnp.uint32).at[:, pl.ds(128 * t, 128)],
                                                 d.at[t, pl.ds(0, s.shape[0] // 2)], sems.at[i, t])
                           for t in range(d.shape[0])])
        else:
            copies.append([pltpu.make_async_copy(s, d, sems.at[i, 0])])

    def start(*ids):
        for i in ids:
            for cp in copies[i]:
                cp.start()

    def wait(*ids):
        for i in ids:
            for cp in copies[i]:
                cp.wait()

    b_scale = Dh ** -0.5 * _LOG2E
    start(6, 8)
    wait(6)
    xb[...] = xbT[...].T
    accT[...] = jnp.zeros_like(accT)
    wait(8)
    start(2, 3, 4, 5, 0, 1)

    def q_pair(i):
        for t, w in enumerate(_head_pair(rbq, i, Dm, HP)):
            qall[2 * i + t] = (_dot(xb[...], w) * b_scale).astype(bf16)

    def q_first(i, _):
        q_pair(i)
        return 0

    def q_second(i, _):
        q_pair(HP - 4 + i)
        wql[2 * i], wql[2 * i + 1] = _head_pair(rbq, HP - 2 + i, Dm, HP)
        for pair in [i * (HP // 2) + u for u in range(HP // 2)]:
            for j, raw in enumerate((rq, rk, rv)):
                for t, w in enumerate(_head_pair(raw, pair, Dm, HP)):
                    wqkv[j * H + 2 * pair + t] = w[0:DK]
                    w4[j * H + 2 * pair + t] = jnp.concatenate([w[DK:, 0:128], w[DK:, 128:]], axis=0)
            tails = []
            for hd in (2 * pair, 2 * pair + 1):
                wo[pl.ds(pl.multiple_of(hd * Dh, Dh), Dh), :] = (
                    woT[pl.ds(pl.multiple_of(hd * Dm, Dm), DK), :].T)
                tails.append(woT[pl.ds(pl.multiple_of(hd * Dm + DK, Dm - DK), Dm - DK), :])
            wo4[pair] = jnp.concatenate(tails, axis=0).T
        return 0

    lax.fori_loop(0, HP - 4, q_first, 0)
    wait(0, 1, 2, 3, 4, 5)
    start(7, 9, 10, 11)
    lax.fori_loop(0, 2, q_second, 0)
    xa[...] = xaT[...].T

    L = seg + M
    row = lax.broadcasted_iota(jnp.int32, (2 * L, 2 * L), 0)
    col = lax.broadcasted_iota(jnp.int32, (2 * L, 2 * L), 1)
    same_head = (row >= L) == (col >= L)
    r = jnp.where(row >= L, row - L, row)
    cc = jnp.where(col >= L, col - L, col)
    keep = same_head & ((cc >= seg) | (r >= seg) | (cc <= r))
    fill = jnp.where(same_head, -1e9 * _LOG2E, -jnp.inf).astype(f32)
    a_scale = Dh ** -0.5 * _LOG2E

    def segment(s, h_head, h_rest, order, late):
        h = jnp.concatenate([h_head[:, 0:DK], h_rest[:, 0:DK].astype(bf16)], axis=0)
        R = h.shape[0]
        h4 = jnp.concatenate([h_head[:, DK:Dm].astype(f32), h_rest[:, DK:Dm]], axis=0)
        z4 = jnp.zeros_like(h4)
        h4 = jnp.concatenate([jnp.concatenate([h4, z4], axis=1),
                              jnp.concatenate([z4, h4], axis=1)], axis=0).astype(bf16)
        qkv, ps, ohs, left = {}, {}, {}, {}

        def proj(g):
            def one(n):
                tail = _dot(h4, w4[n])
                return order(n, _dot(h, wqkv[n]) + jnp.concatenate([tail[0:R], tail[R:]], axis=1))

            def both(j):
                return jnp.concatenate([one(j * H + 2 * g + t) for t in range(2)], axis=0)
            qkv[g] = ((both(0) * a_scale).astype(bf16), both(1).astype(bf16), both(2).astype(bf16))

        def scores(g):
            q, k, _ = qkv[g]
            sc = jnp.where(keep, _dot_nt(q, k), fill)
            e = jnp.exp2(sc - jnp.max(sc, axis=-1, keepdims=True))
            ps[g] = (e / jnp.sum(e, axis=-1, keepdims=True)).astype(bf16)

        def context(g):
            o2 = _dot(ps[g], qkv[g][2])
            for t in range(2):
                oh = o2[t * L:(t + 1) * L]
                if late is None:
                    left[2 * g + t] = oh[seg - M:seg]
                    oh = jnp.concatenate([oh[0:seg - M], oh[seg:L]], axis=0)
                else:
                    oh = jnp.concatenate([oh, late[2 * g + t]], axis=0)
                ohs[2 * g + t] = oh.astype(bf16)

        for g in range(HP):
            proj(g)
            if g >= 1:
                scores(g - 1)
            if g >= 2:
                context(g - 2)
        o = o4 = None
        for t in range(H):
            part = _dot(ohs[t], wo[pl.ds(t * Dh, Dh), :])
            o = part if o is None else o + part
            if t % 2:
                part = _dot(jnp.concatenate([ohs[t - 1], ohs[t]], axis=0), wo4[t // 2])
                o4 = part if o4 is None else o4 + part
            if t == 1:
                scores(HP - 1)
            if t == 3:
                context(HP - 2)
            if t == 6:
                context(HP - 1)
        nrow = 4 * S // (S // seg)
        hd = s // (S // nrow)
        rows = pl.ds(pl.multiple_of(s % (S // nrow) * nrow, nrow), nrow)
        qall[H - 4 + hd, rows, :] = (_dot(xb[rows, :], wql[hd]) * b_scale).astype(bf16)
        RO = o.shape[0]
        return jnp.concatenate([o, o4[0:RO, 0:Dm - DK] + o4[RO:, Dm - DK:]], axis=1), left

    def a_step(i, mem):
        r0 = pl.multiple_of(i * 2 * seg, 2 * seg)
        r1 = pl.multiple_of(r0 + seg, seg)
        ahead = xa[pl.ds(r1, 2 * M), :].astype(f32)
        early = {}

        def order0(n, y):
            early[n] = y[seg:L]
            return jnp.concatenate([y[0:seg], y[L:L + M]], axis=0)

        def order1(n, y):
            n2 = seg - 2 * M
            return jnp.concatenate([early[n], y[n2:n2 + M], y[0:n2], y[n2 + M:seg]], axis=0)

        o0, left = segment(2 * i, xa[pl.ds(r0, seg), :],
                           jnp.concatenate([ahead[0:M], mem], axis=0), order0, None)
        mem = o0[seg - M:seg].astype(bf16).astype(f32)
        o1, _ = segment(2 * i + 1, xa[pl.ds(pl.multiple_of(r1 + 2 * M, 2 * M), seg - 2 * M), :],
                        jnp.concatenate([ahead[M:2 * M], mem], axis=0), order1, left)
        tokens = jnp.concatenate([o0[0:seg - M], o1[L:L + M], o1[0:seg]], axis=0)
        out_ref[pl.ds(r0, 2 * seg), 0:Dm] = tokens.astype(out_ref.dtype)
        return o1[seg:L].astype(bf16).astype(f32)

    lax.fori_loop(0, S // (2 * seg), a_step, mem0[...].astype(f32))

    split = Dm // 128 * 128
    outs = [pltpu.make_async_copy(out_ref.at[:, pl.ds(0, split)], out_hbm.at[:, pl.ds(0, split)], osems.at[4])]
    outs[0].start()
    wait(7, 9, 10, 11)
    HB = BQ // 2
    masked = -1e9 * _LOG2E
    vis_a = (lax.broadcasted_iota(jnp.int32, (BQ, HB), 1)
             <= lax.broadcasted_iota(jnp.int32, (BQ, HB), 0))
    vis_b = vis_a[0:HB]

    def b_pair(i, _):
        wk2 = _head_pair(rbuk, i, Dc, HP)
        wv2 = _head_pair(rbuv, i, Dc, HP)
        for t in range(2):
            hd = 2 * i + t
            ks[...] = _dot(c[...], wk2[t]).astype(bf16)
            vs[...] = _dot(c[...], wv2[t]).astype(bf16)
            w_out = boT[pl.ds(pl.multiple_of(hd * Dm, Dm), Dm), :]
            sc, ctxs = {}, {}
            NQ = S // BQ
            CK = BQ

            def chunks(qb):
                return [(j * CK, min((j + 1) * CK, qb * BQ)) for j in range(-(-qb * BQ // CK))]

            def fold(x, op):
                r = x[:, 0:128]
                for j in range(1, x.shape[1] // 128):
                    r = op(r, x[:, j * 128:(j + 1) * 128])
                return r

            def scores(qb):
                lo, mid, hi = qb * BQ, qb * BQ + HB, (qb + 1) * BQ
                q = qall[hd, lo:hi, :]
                sa = jnp.where(vis_a, _dot_nt(q, ks[lo:mid, :]), masked)
                sb = jnp.where(vis_b, _dot_nt(q[HB:], ks[mid:hi, :]), masked)
                top = jnp.concatenate([sa[0:HB], jnp.maximum(sa[HB:], sb)], axis=0)
                so = []
                yield
                for u, w in chunks(qb):
                    x = _dot_nt(q, ks[u:w, :])
                    top = jnp.maximum(top, fold(x, jnp.maximum))
                    so.append(x)
                    yield
                sc[qb] = (sa, sb, so, jnp.max(top, axis=-1, keepdims=True))

            def context(qb):
                lo, mid, hi = qb * BQ, qb * BQ + HB, (qb + 1) * BQ
                sa, sb, so, m = sc[qb]
                ea = jnp.exp2(sa - m)
                eb = jnp.exp2(sb - m[HB:])
                l = jnp.concatenate([ea[0:HB], ea[HB:] + eb], axis=0)
                ctx = _dot(ea.astype(bf16), vs[lo:mid, :])
                cb = _dot(eb.astype(bf16), vs[mid:hi, :])
                ctx = jnp.concatenate([ctx[0:HB], ctx[HB:] + cb], axis=0)
                yield
                for (u, w), x in zip(chunks(qb), so):
                    e = jnp.exp2(x - m)
                    l = l + fold(e, jnp.add)
                    ctx = ctx + _dot(e.astype(bf16), vs[u:w, :])
                    yield
                ctxs[qb] = (ctx / jnp.sum(l, axis=-1, keepdims=True)).astype(bf16)

            def project(qb):
                for _ in range(max(qb - 1, 0) // 2):
                    yield
                accT[:, qb * BQ:(qb + 1) * BQ] += _dot_nt(w_out, ctxs[qb])
                yield

            def weave(*gens):
                gens = list(gens)
                while gens:
                    for g in list(gens):
                        if next(g, "end") == "end":
                            gens.remove(g)

            order = list(range(NQ))[::-1]
            for step in range(NQ + 2):
                weave(*[fn(order[step - d]) for fn, d in ((scores, 0), (context, 1), (project, 2)) if 0 <= step - d < NQ])
        return 0

    lax.fori_loop(0, HP, b_pair, 0)
    for j in range(4):
        rows = pl.ds(j * (S // 4), S // 4)
        out_ref[rows, Dm:2 * Dm] = accT[:, rows].T.astype(out_ref.dtype)
        cols = pl.ds(split, 2 * Dm - split)
        outs.append(pltpu.make_async_copy(out_ref.at[rows, cols], out_hbm.at[rows, cols], osems.at[j]))
        outs[-1].start()
    for cp in outs:
        cp.wait()


@functools.partial(jax.jit, static_argnames=("A_seg_len",))
def pallas_concat_heads__memory_aug_recurrent_mem_tr__compressed_kv_cla__prompt_kernel(
    A_x, A_mem0, A_Wq, A_Wk, A_Wv, A_Wo, A_seg_len,
    B_x, B_c_kv, B_w_q, B_w_uk, B_w_uv, B_w_o,
):
    _, S, Dm = A_x.shape
    _, H, Dh = A_Wq.shape
    M = A_mem0.shape[1]
    Dc = B_c_kv.shape[2]
    seg = int(A_seg_len)
    bf16 = jnp.bfloat16
    BQ = 256
    DK = Dm // 128 * 128
    args = (
        A_x.reshape(S, Dm).T, A_mem0.reshape(M, Dm),
        A_Wq.reshape(Dm * H, Dh), A_Wk.reshape(Dm * H, Dh), A_Wv.reshape(Dm * H, Dh),
        A_Wo.transpose(0, 2, 1).reshape(H * Dm, Dh),
        B_x.reshape(S, Dm).T, B_c_kv.reshape(S, Dc),
        B_w_q.reshape(Dm * H, Dh), B_w_uk.reshape(Dc * H, Dh), B_w_uv.reshape(Dc * H, Dh),
        B_w_o.transpose(0, 2, 1).reshape(H * Dm, Dh),
    )
    vm = pltpu.VMEM
    bufs = [vm((Dh // 128, a.shape[0] // 2 + H // 2, 128), jnp.uint32) if i in (2, 3, 4, 8, 9, 10) else vm(a.shape, bf16)
            for i, a in enumerate(args)]
    scratch = bufs[:6]
    scratch += [vm((3 * H, DK, Dh), bf16)]
    scratch += bufs[6:]
    scratch += [vm((Dm, S), jnp.float32), vm((H, S, Dh), bf16), vm((S, Dh), bf16), vm((S, Dh), bf16),
                vm((S, Dm), bf16), vm((S, Dm), bf16), vm((H * Dh, DK), bf16),
                vm((3 * H, 128, 128), bf16), vm((H // 2, Dh, 128), bf16), vm((4, Dm, Dh), bf16),
                vm((S, 2 * Dm), bf16),
                pltpu.SemaphoreType.DMA((12, Dh // 128)), pltpu.SemaphoreType.DMA((5,))]
    out = pl.pallas_call(
        functools.partial(_kernel, S=S, Dm=Dm, H=H, Dh=Dh, M=M, seg=seg, Dc=Dc, BQ=BQ),
        out_shape=jax.ShapeDtypeStruct((S, 2 * Dm), bf16),
        in_specs=[pl.BlockSpec(memory_space=pltpu.HBM)] * 12,
        out_specs=pl.BlockSpec(memory_space=pltpu.HBM),
        scratch_shapes=scratch,
        compiler_params=pltpu.CompilerParams(vmem_limit_bytes=120 * 1024 * 1024),
    )(*args)
    return out.reshape(1, S, 2 * Dm)
```
